```python
import jax
import jax.numpy as jnp

def _softmax(x, axis=-1):
    return jax.nn.softmax(x, axis=axis)
def _gelu(x):
    return jax.nn.gelu(x, approximate=True)
def _silu(x):
    return jax.nn.silu(x)
def _sigmoid(x):
    return jax.nn.sigmoid(x)
def _layernorm(x, axis=-1, eps=1e-5):
    m = jnp.mean(x, axis=axis, keepdims=True)
    v = jnp.var(x, axis=axis, keepdims=True)
    return (x - m) / jnp.sqrt(v + eps)
def _scatter_add(tgt, idx, src, axis=0):
    return tgt.at[idx].add(src)
def _segment_sum(src, seg, n):
    return jax.ops.segment_sum(src, seg, n)
class _Rng:
    def __init__(self, key):
        self._k = key
    def _next(self):
        self._k, sub = jax.random.split(self._k)
        return sub
    def normal(self, shape):
        return jax.random.normal(self._next(), shape, dtype=jnp.bfloat16)
    def randint(self, lo, hi, shape):
        return jax.random.randint(self._next(), shape, lo, hi, dtype=jnp.int32)
    def uniform(self, shape, lo=0.0, hi=1.0):
        return jax.random.uniform(self._next(), shape, jnp.bfloat16, lo, hi)
    def permutation(self, n):
        return jax.random.permutation(self._next(), n)


kernel_name = 'standalone__gqa_softmax__near_ridge'

def setup_inputs():
    _rng = _Rng(jax.random.key(int.from_bytes(__import__("os").urandom(4), "little")))
    _w = (lambda a: (lambda t: t.astype(jnp.bfloat16) if jnp.issubdtype(t.dtype, jnp.floating) else t)(jnp.asarray(a)))
    B, Hq, Hkv, Sq, Sk, D = 16, 32, 32, 848, 512, 192
    return {
        "q": _w((lambda *s: _rng.normal(s) * 0.05)(B, Hq, Sq, D)),
        "k": _w((lambda *s: _rng.normal(s) * 0.05)(B, Hkv, Sk, D)),
        "v": _w((lambda *s: _rng.normal(s) * 0.05)(B, Hkv, Sk, D)),
    }

def reference(q, k, v):
    B, Hq, Sq, D = q.shape
    Hkv = k.shape[1]
    rep = Hq // Hkv
    k = jnp.repeat(k, rep, axis=1)
    v = jnp.repeat(v, rep, axis=1)
    scale = D ** -0.5
    scores = jnp.einsum("bhqd,bhkd->bhqk", q, k) * scale
    p = _softmax(scores, axis=-1)
    return jnp.einsum("bhqk,bhkd->bhqd", p, v)
```

```python
import jax
import jax.numpy as jnp
import jax.experimental.pallas as pl
import jax.experimental.pallas.tpu as pltpu

_LOG2E = 1.4426950408889634
_HEADS_PER_STEP = 2


def _attn_kernel(qT_ref, kT_ref, vT_ref, oT_ref):
    hb, D, _ = qT_ref.shape
    c = (D ** -0.5) * _LOG2E
    for h in range(hb):
        k = kT_ref[h].T
        sT = jnp.dot(k, qT_ref[h], preferred_element_type=jnp.float32)
        m = jnp.max(sT, axis=0, keepdims=True)
        p = jnp.exp2((sT - m) * c)
        l = jnp.sum(p, axis=0, keepdims=True)
        oT = jnp.dot(vT_ref[h], p.astype(vT_ref.dtype), preferred_element_type=jnp.float32)
        oT_ref[h] = (oT * (1.0 / l)).astype(oT_ref.dtype)


@jax.jit
def pallas_standalone__gqa_softmax__near_ridge_kernel(
    q: jax.Array,
    k: jax.Array,
    v: jax.Array,
):
    B, H, Sq, D = q.shape
    Sk = k.shape[2]
    assert k.shape[1] == H and v.shape[1] == H
    hb = _HEADS_PER_STEP
    qT = jnp.swapaxes(q, 2, 3).reshape(B * H, D, Sq)
    kT = jnp.swapaxes(k, 2, 3).reshape(B * H, D, Sk)
    vT = jnp.swapaxes(v, 2, 3).reshape(B * H, D, Sk)
    oT = pl.pallas_call(
        _attn_kernel,
        grid=(B * H // hb,),
        in_specs=[
            pl.BlockSpec((hb, D, Sq), lambda i: (i, 0, 0)),
            pl.BlockSpec((hb, D, Sk), lambda i: (i, 0, 0)),
            pl.BlockSpec((hb, D, Sk), lambda i: (i, 0, 0)),
        ],
        out_specs=pl.BlockSpec((hb, D, Sq), lambda i: (i, 0, 0)),
        out_shape=jax.ShapeDtypeStruct((B * H, D, Sq), q.dtype),
        compiler_params=pltpu.CompilerParams(
            dimension_semantics=("parallel",),
            vmem_limit_bytes=64 * 1024 * 1024,
        ),
    )(qT, kT, vT)
    return jnp.swapaxes(oT.reshape(B, H, D, Sq), 2, 3)
```

```python
import jax
import jax.numpy as jnp
from jax import lax
import jax.experimental.pallas as pl
import jax.experimental.pallas.tpu as pltpu

_LOG2E = 1.4426950408889634
_HEADS_PER_STEP = 8
_COL_CHUNK = 384
_SKEW = 2
_NT = (((1,), (1,)), ((), ()))


def _attn_kernel(qT_ref, kT_ref, vT_ref, oT_ref):
    hb, D, Sq = qT_ref.shape
    c = (D ** -0.5) * _LOG2E
    main = (Sq // _COL_CHUNK) * _COL_CHUNK

    units = []
    for h in range(hb):
        if main < Sq:
            units.append((h, main, Sq - main, False))
        units.extend((h, st, _COL_CHUNK, True) for st in range(0, main, _COL_CHUNK))

    k_rows = {}
    scores = {}

    def qk(u):
        h, st, w, on_lanes = units[u]
        if on_lanes:
            if h not in k_rows:
                k_rows[h] = kT_ref[h].T
            scores[u] = jnp.dot(k_rows[h], qT_ref[h, :, st:st + w], preferred_element_type=jnp.float32)
        else:
            scores[u] = jnp.dot(qT_ref[h, :, st:st + w].T, kT_ref[h], preferred_element_type=jnp.float32)

    def softmax_pv(u):
        h, st, w, on_lanes = units[u]
        s = scores.pop(u)
        axis = 0 if on_lanes else 1
        m = jnp.max(s, axis=axis, keepdims=True)
        p = jnp.exp2((s - m) * c)
        inv_l = 1.0 / jnp.sum(p, axis=axis, keepdims=True)
        p = p.astype(vT_ref.dtype)
        if on_lanes:
            oT = jnp.dot(vT_ref[h], p, preferred_element_type=jnp.float32)
            oT_ref[h, :, st:st + w] = (oT * inv_l).astype(oT_ref.dtype)
        else:
            o = lax.dot_general(p, vT_ref[h], _NT, preferred_element_type=jnp.float32)
            oT_ref[h, :, st:st + w] = (o * inv_l).astype(oT_ref.dtype).T

    for t in range(len(units) + _SKEW):
        if t < len(units):
            qk(t)
        if t >= _SKEW:
            softmax_pv(t - _SKEW)


@jax.jit
def pallas_standalone__gqa_softmax__near_ridge_kernel(
    q: jax.Array,
    k: jax.Array,
    v: jax.Array,
):
    B, H, Sq, D = q.shape
    Sk = k.shape[2]
    assert k.shape[1] == H and v.shape[1] == H
    hb = _HEADS_PER_STEP
    qT = jnp.swapaxes(q, 2, 3).reshape(B * H, D, Sq)
    kT = jnp.swapaxes(k, 2, 3).reshape(B * H, D, Sk)
    vT = jnp.swapaxes(v, 2, 3).reshape(B * H, D, Sk)
    oT = pl.pallas_call(
        _attn_kernel,
        grid=(B * H // hb,),
        in_specs=[
            pl.BlockSpec((hb, D, Sq), lambda i: (i, 0, 0)),
            pl.BlockSpec((hb, D, Sk), lambda i: (i, 0, 0)),
            pl.BlockSpec((hb, D, Sk), lambda i: (i, 0, 0)),
        ],
        out_specs=pl.BlockSpec((hb, D, Sq), lambda i: (i, 0, 0)),
        out_shape=jax.ShapeDtypeStruct((B * H, D, Sq), q.dtype),
        compiler_params=pltpu.CompilerParams(
            dimension_semantics=("parallel",),
            vmem_limit_bytes=64 * 1024 * 1024,
            flags={"XLA_TPU_FORCE_LP_LLO_SCHEDULER": True},
        ),
    )(qT, kT, vT)
    return jnp.swapaxes(oT.reshape(B, H, D, Sq), 2, 3)
```

```python
import jax
import jax.numpy as jnp
from jax import lax
import jax.experimental.pallas as pl
import jax.experimental.pallas.tpu as pltpu

_LOG2E = 1.4426950408889634
_LANES = 128
_GROUP = 16
_PIECE = 2
_CHUNK = 384
_SKEW = 2
_NT = (((1,), (1,)), ((), ()))


def _heads(q_ref, k_ref, v_ref, o_ref, k_carry):
    n, D, Sq = q_ref.shape
    dt = v_ref.dtype
    c = (D ** -0.5) * _LOG2E
    main = Sq - Sq % _LANES
    d_split = D - D % _LANES

    units = []
    for h in range(n):
        cols = [(h, st, min(_CHUNK, main - st), True) for st in range(0, main, _CHUNK)]
        units += cols[:1] + [(h, main, Sq - main, False)] + cols[1:]

    k_rows = {0: pltpu.bitcast(k_carry[...], dt)}
    scores = {}

    def qk(u):
        h, st, w, on_lanes = units[u]
        q = q_ref[h, :, st:st + w]
        if on_lanes:
            if h not in k_rows:
                k_rows[h] = k_ref[h].T
            scores[u] = jnp.dot(k_rows[h], q, preferred_element_type=jnp.float32)
        else:
            scores[u] = jnp.dot(q.T, k_ref[h], preferred_element_type=jnp.float32)

    def softmax_pv(u):
        h, st, w, on_lanes = units[u]
        s = scores.pop(u)
        axis = 0 if on_lanes else 1
        m = jnp.max(s, axis=axis, keepdims=True)
        p = jnp.exp2((s - m) * c)
        if on_lanes:
            p_lo = p.astype(dt)
            l = jnp.sum(p, axis=0, keepdims=True)
            o = jnp.dot(v_ref[h], p_lo, preferred_element_type=jnp.float32)
            o_ref[h, :, st:st + w] = (o * (1.0 / l)).astype(o_ref.dtype)
        else:
            l = jnp.sum(p, axis=1, keepdims=True)
            p_lo = (p * (1.0 / l)).astype(dt)
            o = lax.dot_general(p_lo, v_ref[h, :d_split], _NT, preferred_element_type=jnp.float32)
            o_ref[h, :d_split, st:st + w] = o.astype(o_ref.dtype).T
            o = lax.dot_general(v_ref[h, d_split:], p_lo, _NT, preferred_element_type=jnp.float32)
            o_ref[h, d_split:, st:st + w] = o.astype(o_ref.dtype)

    for t in range(len(units) + _SKEW):
        if t < len(units):
            qk(t)
        if t == len(units) - 1:
            k_carry[...] = pltpu.bitcast(k_ref[n].T, k_carry.dtype)
        if t >= _SKEW:
            softmax_pv(t - _SKEW)


def _attn_kernel(q_hbm, k_hbm, v_hbm, o_hbm, qb, kb, vb, ob, k_carry, sems, piece_sems):
    N = q_hbm.shape[0]
    G, g = _GROUP, _PIECE
    n_blocks, n_pieces = N // G, G // g

    def compute(slot, h0, cnt):
        _heads(
            qb.at[slot, pl.ds(h0, cnt)],
            kb.at[slot, pl.ds(h0, cnt + 1)],
            vb.at[slot, pl.ds(h0, cnt)],
            ob.at[slot, pl.ds(h0, cnt)],
            k_carry,
        )

    def piece_loads(blk, j, sem):
        h0 = j * g
        src = blk * G + h0
        return [
            pltpu.make_async_copy(k_hbm.at[pl.ds(src + 1, g)], kb.at[blk, pl.ds(h0 + 1, g)], sem.at[1]),
            pltpu.make_async_copy(q_hbm.at[pl.ds(src, g)], qb.at[blk, pl.ds(h0, g)], sem.at[0]),
            pltpu.make_async_copy(v_hbm.at[pl.ds(src, g)], vb.at[blk, pl.ds(h0, g)], sem.at[2]),
        ]

    def first_k(blk):
        return pltpu.make_async_copy(k_hbm.at[blk * G], kb.at[blk, 0], sems.at[blk, 1])

    def start_block_load(blk, slot):
        sem = sems.at[slot]
        heads = pl.ds(blk * G, G)
        after = jnp.minimum(blk * G + G, N - 1)
        pltpu.make_async_copy(q_hbm.at[heads], qb.at[slot], sem.at[0]).start()
        pltpu.make_async_copy(k_hbm.at[heads], kb.at[slot, pl.ds(0, G)], sem.at[1]).start()
        pltpu.make_async_copy(k_hbm.at[after], kb.at[slot, G], sem.at[1]).start()
        pltpu.make_async_copy(v_hbm.at[heads], vb.at[slot], sem.at[2]).start()

    def wait_block_load(slot):
        for i, buf in enumerate((qb, kb, vb)):
            pltpu.make_async_copy(buf.at[slot], buf.at[slot], sems.at[slot, i]).wait()

    def store(blk, slot, h0, cnt):
        return pltpu.make_async_copy(
            ob.at[slot, pl.ds(h0, cnt)], o_hbm.at[pl.ds(blk * G + h0, cnt)], sems.at[slot, 3]
        )

    first_k(0).start()
    for j in range(2):
        for cp in piece_loads(0, j, piece_sems.at[j]):
            cp.start()
    first_k(1).start()
    first_k(0).wait()
    k_carry[...] = pltpu.bitcast(kb[0, 0].T, k_carry.dtype)

    def fill(j, carry):
        for cp in piece_loads(0, j, piece_sems.at[j]):
            cp.wait()

        @pl.when(j + 2 < n_pieces)
        def _():
            for cp in piece_loads(0, j + 2, piece_sems.at[j + 2]):
                cp.start()

        for cp in piece_loads(1, j, sems.at[1]):
            cp.start()
        compute(0, j * g, g)
        return carry

    lax.fori_loop(0, n_pieces, fill, 0)
    store(0, 0, 0, G).start()

    def steady(i, carry):
        slot = i % 2
        wait_block_load(slot)
        start_block_load(i + 1, 1 - slot)

        @pl.when(i >= 2)
        def _():
            store(i - 2, slot, 0, G).wait()

        compute(slot, 0, G)
        store(i, slot, 0, G).start()
        return carry

    lax.fori_loop(1, n_blocks - 1, steady, 0)

    last = n_blocks - 1
    wait_block_load(1)
    store(last - 2, 1, 0, G).wait()

    def drain(j, carry):
        compute(1, j * g, g)
        store(last, 1, j * g, g).start()
        return carry

    lax.fori_loop(0, n_pieces, drain, 0)
    store(last - 1, 0, 0, G).wait()
    store(last, 1, 0, G).wait()


@jax.jit
def pallas_standalone__gqa_softmax__near_ridge_kernel(
    q: jax.Array,
    k: jax.Array,
    v: jax.Array,
):
    B, H, Sq, D = q.shape
    Sk = k.shape[2]
    N, G = B * H, _GROUP
    assert k.shape == v.shape == (B, H, Sk, D)
    assert N % (2 * G) == 0 and N >= 4 * G
    qT = jnp.swapaxes(q, 2, 3).reshape(N, D, Sq)
    kT = jnp.swapaxes(k, 2, 3).reshape(N, D, Sk)
    vT = jnp.swapaxes(v, 2, 3).reshape(N, D, Sk)
    oT = pl.pallas_call(
        _attn_kernel,
        in_specs=[pl.BlockSpec(memory_space=pl.ANY)] * 3,
        out_specs=pl.BlockSpec(memory_space=pl.ANY),
        out_shape=jax.ShapeDtypeStruct((N, D, Sq), q.dtype),
        scratch_shapes=[
            pltpu.VMEM((2, G, D, Sq), q.dtype),
            pltpu.VMEM((2, G + 1, D, Sk), k.dtype),
            pltpu.VMEM((2, G, D, Sk), v.dtype),
            pltpu.VMEM((2, G, D, Sq), q.dtype),
            pltpu.VMEM((Sk // 2, D), jnp.uint32),
            pltpu.SemaphoreType.DMA((2, 4)),
            pltpu.SemaphoreType.DMA((G // _PIECE, 3)),
        ],
        compiler_params=pltpu.CompilerParams(
            vmem_limit_bytes=100 * 1024 * 1024,
            disable_bounds_checks=True,
            flags={"XLA_TPU_FORCE_LP_LLO_SCHEDULER": True},
        ),
    )(qT, kT, vT)
    return jnp.swapaxes(oT.reshape(B, H, D, Sq), 2, 3)
```

```python
import jax
import jax.numpy as jnp
from jax import lax
import jax.experimental.pallas as pl
import jax.experimental.pallas.tpu as pltpu

_LOG2E = 1.4426950408889634
_LANES = 128
_GROUP = 16
_PIECE = 2
_NT = (((1,), (1,)), ((), ()))

_COL_TILES = 6
_ORDER = (
    ("qk", 0, 3, 0),
    ("pv", 3, 4, 1),
    ("qk_rest", 0, 0, 0),
    ("pv", 4, 6, 1),
    ("qk", 3, 6, 0),
    ("pv_rest", 0, 0, 0),
    ("pv", 0, 3, 0),
)


def _heads(q_ref, k_ref, v_ref, o_ref, k_carry):
    n, D, Sq = q_ref.shape
    dt = v_ref.dtype
    c = (D ** -0.5) * _LOG2E
    rest = _COL_TILES * _LANES
    d_split = D - D % _LANES

    k_rows = {0: pltpu.bitcast(k_carry[...], dt)}
    scores = {}

    def qk(h, lo, hi):
        if h not in k_rows:
            k_rows[h] = k_ref[h].T
        q = q_ref[h, :, lo * _LANES:hi * _LANES]
        s = jnp.dot(k_rows[h], q, preferred_element_type=jnp.float32)
        for j in range(lo, hi):
            scores[h, j] = (s, lo)

    def pv(h, lo, hi):
        s, first = scores[h, lo]
        s = s[:, (lo - first) * _LANES:(hi - first) * _LANES]
        m = jnp.max(s, axis=0, keepdims=True)
        p = jnp.exp2((s - m) * c)
        p_lo = p.astype(dt)
        l = jnp.sum(p, axis=0, keepdims=True)
        o = jnp.dot(v_ref[h], p_lo, preferred_element_type=jnp.float32)
        o_ref[h, :, lo * _LANES:hi * _LANES] = (o * (1.0 / l)).astype(o_ref.dtype)

    def qk_rest(h):
        q = q_ref[h, :, rest:].T
        scores[h] = jnp.dot(q, k_ref[h], preferred_element_type=jnp.float32)

    def pv_rest(h):
        s = scores[h]
        m = jnp.max(s, axis=1, keepdims=True)
        p = jnp.exp2((s - m) * c)
        l = jnp.sum(p, axis=1, keepdims=True)
        p_lo = (p * (1.0 / l)).astype(dt)
        o = lax.dot_general(p_lo, v_ref[h, :d_split], _NT, preferred_element_type=jnp.float32)
        o_ref[h, :d_split, rest:] = o.astype(o_ref.dtype).T
        o = lax.dot_general(v_ref[h, d_split:], p_lo, _NT, preferred_element_type=jnp.float32)
        o_ref[h, d_split:, rest:] = o.astype(o_ref.dtype)

    for t in range(n + 1):
        for op, lo, hi, lag in _ORDER:
            h = t - lag
            if not 0 <= h < n:
                continue
            if op == "qk":
                qk(h, lo, hi)
                if h == n - 1 and hi == _COL_TILES:
                    k_carry[...] = pltpu.bitcast(k_ref[n].T, k_carry.dtype)
            elif op == "pv":
                pv(h, lo, hi)
            elif op == "qk_rest":
                qk_rest(h)
            else:
                pv_rest(h)


def _attn_kernel(q_hbm, k_hbm, v_hbm, o_hbm, qb, kb, vb, ob, k_carry, sems, piece_sems):
    N = q_hbm.shape[0]
    G, g = _GROUP, _PIECE
    n_blocks, n_pieces = N // G, G // g

    def compute(slot, h0, cnt):
        _heads(
            qb.at[slot, pl.ds(h0, cnt)],
            kb.at[slot, pl.ds(h0, cnt + 1)],
            vb.at[slot, pl.ds(h0, cnt)],
            ob.at[slot, pl.ds(h0, cnt)],
            k_carry,
        )

    def piece_loads(blk, j, sem):
        h0 = j * g
        src = blk * G + h0
        return [
            pltpu.make_async_copy(k_hbm.at[pl.ds(src + 1, g)], kb.at[blk, pl.ds(h0 + 1, g)], sem.at[1]),
            pltpu.make_async_copy(q_hbm.at[pl.ds(src, g)], qb.at[blk, pl.ds(h0, g)], sem.at[0]),
            pltpu.make_async_copy(v_hbm.at[pl.ds(src, g)], vb.at[blk, pl.ds(h0, g)], sem.at[2]),
        ]

    def first_k(blk):
        return pltpu.make_async_copy(k_hbm.at[blk * G], kb.at[blk, 0], sems.at[blk, 1])

    def start_block_load(blk, slot):
        sem = sems.at[slot]
        heads = pl.ds(blk * G, G)
        after = jnp.minimum(blk * G + G, N - 1)
        pltpu.make_async_copy(q_hbm.at[heads], qb.at[slot], sem.at[0]).start()
        pltpu.make_async_copy(k_hbm.at[heads], kb.at[slot, pl.ds(0, G)], sem.at[1]).start()
        pltpu.make_async_copy(k_hbm.at[after], kb.at[slot, G], sem.at[1]).start()
        pltpu.make_async_copy(v_hbm.at[heads], vb.at[slot], sem.at[2]).start()

    def wait_block_load(slot):
        for i, buf in enumerate((qb, kb, vb)):
            pltpu.make_async_copy(buf.at[slot], buf.at[slot], sems.at[slot, i]).wait()

    def store(blk, slot, h0, cnt):
        return pltpu.make_async_copy(
            ob.at[slot, pl.ds(h0, cnt)], o_hbm.at[pl.ds(blk * G + h0, cnt)], sems.at[slot, 3]
        )

    first_k(0).start()
    for j in range(2):
        for cp in piece_loads(0, j, piece_sems.at[j]):
            cp.start()
    first_k(1).start()
    first_k(0).wait()
    k_carry[...] = pltpu.bitcast(kb[0, 0].T, k_carry.dtype)

    def fill(j, carry):
        for cp in piece_loads(0, j, piece_sems.at[j]):
            cp.wait()

        @pl.when(j + 2 < n_pieces)
        def _():
            for cp in piece_loads(0, j + 2, piece_sems.at[j + 2]):
                cp.start()

        for cp in piece_loads(1, j, sems.at[1]):
            cp.start()
        compute(0, j * g, g)
        return carry

    lax.fori_loop(0, n_pieces, fill, 0)
    store(0, 0, 0, G).start()

    def steady(i, carry):
        slot = i % 2
        wait_block_load(slot)
        start_block_load(i + 1, 1 - slot)

        @pl.when(i >= 2)
        def _():
            store(i - 2, slot, 0, G).wait()

        compute(slot, 0, G)
        store(i, slot, 0, G).start()
        return carry

    lax.fori_loop(1, n_blocks - 1, steady, 0)

    last = n_blocks - 1
    wait_block_load(1)
    store(last - 2, 1, 0, G).wait()

    def drain(j, carry):
        compute(1, j * g, g)
        store(last, 1, j * g, g).start()
        return carry

    lax.fori_loop(0, n_pieces, drain, 0)
    store(last - 1, 0, 0, G).wait()
    store(last, 1, 0, G).wait()


@jax.jit
def pallas_standalone__gqa_softmax__near_ridge_kernel(
    q: jax.Array,
    k: jax.Array,
    v: jax.Array,
):
    B, H, Sq, D = q.shape
    Sk = k.shape[2]
    N, G = B * H, _GROUP
    assert k.shape == v.shape == (B, H, Sk, D)
    assert N % (2 * G) == 0 and N >= 4 * G
    assert Sq // _LANES == _COL_TILES and Sq % _LANES and D > _LANES and D % _LANES
    qT = jnp.swapaxes(q, 2, 3).reshape(N, D, Sq)
    kT = jnp.swapaxes(k, 2, 3).reshape(N, D, Sk)
    vT = jnp.swapaxes(v, 2, 3).reshape(N, D, Sk)
    oT = pl.pallas_call(
        _attn_kernel,
        in_specs=[pl.BlockSpec(memory_space=pl.ANY)] * 3,
        out_specs=pl.BlockSpec(memory_space=pl.ANY),
        out_shape=jax.ShapeDtypeStruct((N, D, Sq), q.dtype),
        scratch_shapes=[
            pltpu.VMEM((2, G, D, Sq), q.dtype),
            pltpu.VMEM((2, G + 1, D, Sk), k.dtype),
            pltpu.VMEM((2, G, D, Sk), v.dtype),
            pltpu.VMEM((2, G, D, Sq), q.dtype),
            pltpu.VMEM((Sk // 2, D), jnp.uint32),
            pltpu.SemaphoreType.DMA((2, 4)),
            pltpu.SemaphoreType.DMA((G // _PIECE, 3)),
        ],
        compiler_params=pltpu.CompilerParams(
            vmem_limit_bytes=100 * 1024 * 1024,
            disable_bounds_checks=True,
            flags={"XLA_TPU_FORCE_LP_LLO_SCHEDULER": True},
        ),
    )(qT, kT, vT)
    return jnp.swapaxes(oT.reshape(B, H, D, Sq), 2, 3)
```
